```python
import os as _os
_os.environ.setdefault("JAX_PLATFORMS", "cpu")
import jax
import jax.numpy as jnp

def _softmax(x, axis=-1):
    return jax.nn.softmax(x, axis=axis)
def _gelu(x):
    return jax.nn.gelu(x, approximate=True)
def _silu(x):
    return jax.nn.silu(x)
def _sigmoid(x):
    return jax.nn.sigmoid(x)
def _layernorm(x, axis=-1, eps=1e-5):
    m = jnp.mean(x, axis=axis, keepdims=True)
    v = jnp.var(x, axis=axis, keepdims=True)
    return (x - m) / jnp.sqrt(v + eps)
def _scatter_add(tgt, idx, src, axis=0):
    return tgt.at[idx].add(src)
def _segment_sum(src, seg, n):
    return jax.ops.segment_sum(src, seg, n)
class _Rng:
    def __init__(self, key):
        self._k = key
    def _next(self):
        self._k, sub = jax.random.split(self._k)
        return sub
    def normal(self, shape):
        return jax.random.normal(self._next(), shape, dtype=jnp.bfloat16)
    def randint(self, lo, hi, shape):
        return jax.random.randint(self._next(), shape, lo, hi, dtype=jnp.int32)
    def uniform(self, shape, lo=0.0, hi=1.0):
        return jax.random.uniform(self._next(), shape, jnp.bfloat16, lo, hi)
    def permutation(self, n):
        return jax.random.permutation(self._next(), n)


kernel_name = 'sequential_preLN__linear_attn_block__glu_gated_reglu__prompt'

def setup_inputs():
    _rng = _Rng(jax.random.key(int.from_bytes(__import__("os").urandom(4), "little")))
    _w = (lambda a: (lambda t: t.astype(jnp.bfloat16) if jnp.issubdtype(t.dtype, jnp.floating) else t)(jnp.asarray(a)))
    def _A_setup():
        B, S, D = 1, 2048, 640
        return {
            "x": _w((lambda *s: _rng.normal(s) * 0.05)(B, S, D)),
            "wqkv": _w((lambda *s: _rng.normal(s) * 0.05)(D, 3 * D)),
            "wo": _w((lambda *s: _rng.normal(s) * 0.05)(D, D)),
        }
    _A_in = _A_setup()

    def _B_setup():
        B, S, D, F = 1, 2048, 640, 1536
        return {
            "x": _w((lambda *s: _rng.normal(s) * 0.05)(B, S, D)),
            "W_gate": _w((lambda *s: _rng.normal(s) * 0.05)(D, F) * (2.0 / D) ** 0.5),
            "W_up": _w((lambda *s: _rng.normal(s) * 0.05)(D, F) * (2.0 / D) ** 0.5),
            "W_down": _w((lambda *s: _rng.normal(s) * 0.05)(F, D) * (1.0 / F) ** 0.5),
        }
    _B_in = _B_setup()

    return {
        "A_x": _A_in["x"],
        "A_wqkv": _A_in["wqkv"],
        "A_wo": _A_in["wo"],
        "B_x": _B_in["x"],
        "B_W_gate": _B_in["W_gate"],
        "B_W_up": _B_in["W_up"],
        "B_W_down": _B_in["W_down"],
    }

def reference(A_x, A_wqkv, A_wo, B_x, B_W_gate, B_W_up, B_W_down):
    def _A_ref(x, wqkv, wo):
        B, S, D = x.shape
        H = 32; Dh = D // H
        qkv = (lambda x, *d: x.transpose(*d))((x @ wqkv).reshape(B, S, 3, H, Dh), 2, 0, 3, 1, 4)
        q, k, v = qkv[0], qkv[1], qkv[2]
        phi = lambda t: jnp.where(t > 0, t + 1, jnp.exp(t)) + 1e-6
        pq, pk = phi(q), phi(k)
        kv = jnp.einsum("bhsd,bhse->bhde", pk, v)
        z = jnp.einsum("bhsd->bhd", pk)
        num = jnp.einsum("bhqd,bhde->bhqe", pq, kv)
        den = jnp.einsum("bhqd,bhd->bhq", pq, z)[..., None] + 1e-6
        o = num / den
        return (lambda x, *d: x.transpose(*d))(o, 0, 2, 1, 3).reshape(B, S, D) @ wo

    def _B_ref(x, W_gate, W_up, W_down):
        gate = jnp.einsum("bsd,df->bsf", x, W_gate)
        up = jnp.einsum("bsd,df->bsf", x, W_up)
        gate = gate * (lambda x, dt: x.astype(dt))(gate > 0, gate.dtype)
        h = gate * up
        return jnp.einsum("bsf,fd->bsd", h, W_down)

    x = A_x
    h = x + _A_ref(_layernorm(x, axis=-1), A_wqkv, A_wo)
    h2 = h + _B_ref(_layernorm(h, axis=-1), B_W_gate, B_W_up, B_W_down)
    return h2
```

```python
import functools
import jax
import jax.numpy as jnp
from jax import lax
import jax.experimental.pallas as pl
import jax.experimental.pallas.tpu as pltpu

S, D, F, H = 2048, 640, 1536, 32
DH = D // H
TM1 = 512
TM2 = 512
NB1 = S // TM1
NB2 = S // TM2
EPS = 1e-5
bf16 = jnp.bfloat16
f32 = jnp.float32


def _ln(x):
    mu = jnp.mean(x, axis=-1, keepdims=True)
    xc = x - mu
    var = jnp.mean(xc * xc, axis=-1, keepdims=True)
    return xc * lax.rsqrt(var + EPS)


def _phi(t):
    return jnp.where(t > 0, t + 1.0, jnp.exp(t)) + 1e-6


def _head_of(idx):
    return (idx * 3277) >> 16


def _kernel(x_hbm, wqkv_hbm, wo_hbm, wg_hbm, wu_hbm, wd_hbm, out_hbm,
            x_v, wq_v, wk_v, wv_v, wo_v, wg_v, wu_v, wd_v,
            wkt_v, xn_v, g_v, zacc_v, m_v, zc_v, e_v, obuf,
            xsem, wsem, osem):
    def x_copy(i):
        return pltpu.make_async_copy(
            x_hbm.at[pl.ds(i * TM1, TM1), :], x_v.at[pl.ds(i * TM1, TM1), :], xsem.at[i])

    w_copies = [
        pltpu.make_async_copy(wqkv_hbm.at[:, pl.ds(D, D)], wk_v, wsem.at[0]),
        pltpu.make_async_copy(wqkv_hbm.at[:, pl.ds(2 * D, D)], wv_v, wsem.at[1]),
        pltpu.make_async_copy(wo_hbm, wo_v, wsem.at[2]),
        pltpu.make_async_copy(wqkv_hbm.at[:, pl.ds(0, D)], wq_v, wsem.at[3]),
        pltpu.make_async_copy(wg_hbm, wg_v, wsem.at[4]),
        pltpu.make_async_copy(wu_hbm, wu_v, wsem.at[5]),
        pltpu.make_async_copy(wd_hbm, wd_v, wsem.at[6]),
    ]
    x_copy(0).start()
    w_copies[0].start()
    for i in range(1, NB1):
        x_copy(i).start()
    for c in w_copies[1:]:
        c.start()

    g_v[...] = jnp.zeros_like(g_v)
    zacc_v[...] = jnp.zeros_like(zacc_v)

    w_copies[0].wait()
    wkt_v[...] = wk_v[...].astype(f32).T.astype(bf16)

    def p1(i, carry):
        x_copy(i).wait()
        r0 = pl.multiple_of(i * TM1, TM1)
        x = x_v[pl.ds(r0, TM1), :].astype(f32)
        xn = _ln(x).astype(bf16)
        xn_v[pl.ds(r0, TM1), :] = xn
        kt = lax.dot_general(wkt_v[...], xn, (((1,), (1,)), ((), ())),
                             preferred_element_type=f32)
        pkt = _phi(kt)
        za = zacc_v[...]
        for j in range(TM1 // 128):
            za = za + pkt[:, j * 128:(j + 1) * 128]
        zacc_v[...] = za
        g_v[...] += jnp.dot(pkt.astype(bf16), xn, preferred_element_type=f32)
        return carry

    lax.fori_loop(0, NB1, p1, 0)

    w_copies[1].wait()
    w_copies[2].wait()
    rows = lax.broadcasted_iota(jnp.int32, (D, D), 0)
    cols = lax.broadcasted_iota(jnp.int32, (D, D), 1)
    kv = jnp.dot(g_v[...].astype(bf16), wv_v[...], preferred_element_type=f32)
    kv = jnp.where(_head_of(rows) == _head_of(cols), kv, 0.0).astype(bf16)
    m_v[...] = jnp.dot(kv, wo_v[...], preferred_element_type=f32).astype(bf16)

    z = jnp.sum(zacc_v[...], axis=1, keepdims=True)
    r2 = lax.broadcasted_iota(jnp.int32, (D, 128), 0)
    c2 = lax.broadcasted_iota(jnp.int32, (D, 128), 1)
    hz = _head_of(r2)
    zc_v[...] = jnp.where((c2 == hz) | (c2 == hz + H), z, 0.0).astype(bf16)
    r3 = lax.broadcasted_iota(jnp.int32, (128, D), 0)
    c3 = lax.broadcasted_iota(jnp.int32, (128, D), 1)
    he = _head_of(c3)
    e_v[...] = jnp.where((r3 == he) | (r3 == he + H), 1.0, 0.0).astype(bf16)

    for c in w_copies[3:]:
        c.wait()

    def o_copy(i, slot):
        return pltpu.make_async_copy(
            obuf.at[slot], out_hbm.at[pl.ds(i * TM2, TM2), :], osem.at[slot])

    def p2(i, carry):
        slot = i % 2
        r0 = pl.multiple_of(i * TM2, TM2)
        xn = xn_v[pl.ds(r0, TM2), :]
        q = jnp.dot(xn, wq_v[...], preferred_element_type=f32)
        pq = _phi(q)
        den = jnp.dot(pq.astype(bf16), zc_v[...], preferred_element_type=f32) + 1e-6
        r = 1.0 / den
        r_hi = r.astype(bf16)
        r_lo = (r - r_hi.astype(f32)).astype(bf16)
        lane = lax.broadcasted_iota(jnp.int32, (TM2, 128), 1)
        rr = jnp.where(lane < H, r_hi, jnp.where(lane < 2 * H, r_lo, jnp.zeros_like(r_lo)))
        rexp = jnp.dot(rr, e_v[...], preferred_element_type=f32)
        pqn = (pq * rexp).astype(bf16)
        attn = jnp.dot(pqn, m_v[...], preferred_element_type=f32)
        h = x_v[pl.ds(r0, TM2), :].astype(f32) + attn
        hn = _ln(h).astype(bf16)
        g = jnp.dot(hn, wg_v[...], preferred_element_type=f32)
        u = jnp.dot(hn, wu_v[...], preferred_element_type=f32)
        a = (jnp.maximum(g, 0.0) * u).astype(bf16)
        y = jnp.dot(a, wd_v[...], preferred_element_type=f32)

        @pl.when(i >= 2)
        def _():
            o_copy(i - 2, slot).wait()

        obuf[slot] = (h + y).astype(bf16)
        o_copy(i, slot).start()
        return carry

    lax.fori_loop(0, NB2, p2, 0)
    for i in range(max(NB2 - 2, 0), NB2):
        o_copy(i, i % 2).wait()


@jax.jit
def pallas_sequential_preLN__linear_attn_block__glu_gated_reglu__prompt_kernel(
    A_x, A_wqkv, A_wo, B_x, B_W_gate, B_W_up, B_W_down,
):
    x = A_x.reshape(S, D)
    any_spec = pl.BlockSpec(memory_space=pl.ANY)
    out = pl.pallas_call(
        _kernel,
        out_shape=jax.ShapeDtypeStruct((S, D), bf16),
        in_specs=[any_spec] * 6,
        out_specs=any_spec,
        scratch_shapes=[
            pltpu.VMEM((S, D), bf16),
            pltpu.VMEM((D, D), bf16),
            pltpu.VMEM((D, D), bf16),
            pltpu.VMEM((D, D), bf16),
            pltpu.VMEM((D, D), bf16),
            pltpu.VMEM((D, F), bf16),
            pltpu.VMEM((D, F), bf16),
            pltpu.VMEM((F, D), bf16),
            pltpu.VMEM((D, D), bf16),
            pltpu.VMEM((S, D), bf16),
            pltpu.VMEM((D, D), f32),
            pltpu.VMEM((D, 128), f32),
            pltpu.VMEM((D, D), bf16),
            pltpu.VMEM((D, 128), bf16),
            pltpu.VMEM((128, D), bf16),
            pltpu.VMEM((2, TM2, D), bf16),
            pltpu.SemaphoreType.DMA((NB1,)),
            pltpu.SemaphoreType.DMA((7,)),
            pltpu.SemaphoreType.DMA((2,)),
        ],
        compiler_params=pltpu.CompilerParams(vmem_limit_bytes=100 * 1024 * 1024),
    )(x, A_wqkv, A_wo, B_W_gate, B_W_up, B_W_down)
    return out.reshape(1, S, D)
```

```python
import functools
import jax
import jax.numpy as jnp
from jax import lax
import jax.experimental.pallas as pl
import jax.experimental.pallas.tpu as pltpu

S, D, F, H = 2048, 640, 1536, 32
DH = D // H
TM = 512
NB = S // TM
CH = 32
EPS = 1e-5
bf16 = jnp.bfloat16
f32 = jnp.float32
BANDS = [(0, 144), (112, 272), (240, 400), (368, 528), (496, 640)]
GSPLIT = 256
FSPLIT = 768
NT = (((1,), (1,)), ((), ()))
NL = D // 128
WKC = [(0, 256), (256, 384)]
XP = [(0, 256), (256, 256), (512, 512), (1024, 1024)]
OC = [(0, 256), (256, 256), (512, 128)]


def _ln(x):
    mu = jnp.mean(x, axis=-1, keepdims=True)
    xc = x - mu
    var = jnp.mean(xc * xc, axis=-1, keepdims=True)
    return xc * lax.rsqrt(var + EPS)


def _phi(t):
    return jnp.where(t > 0, t + 1.0, jnp.exp(t)) + 1e-6


def _head_of(idx):
    return (idx * 3277) >> 16


def _dot(a, b):
    return jnp.dot(a, b, preferred_element_type=f32)


def _kernel(x_hbm, wqkv_hbm, wo_hbm, wg_hbm, wu_hbm, wd_hbm, out_hbm,
            x_v, wq_v, wk_v, wv_v, wo_v, wg_v, wu_v, wd_v,
            wkt_v, t_v, wqp_v, xn_v, g_v, zacc_v, zp_v, macc_v, m_v,
            pqn_v, at_v, hn_v, obuf,
            sem, osem):
    def xcopy(lo, n, k):
        return pltpu.make_async_copy(x_hbm.at[pl.ds(lo, n), :], x_v.at[pl.ds(lo, n), :], sem.at[k])

    c_x = [xcopy(lo, n, k) for k, (lo, n) in enumerate(XP)]
    c_wk = [pltpu.make_async_copy(wqkv_hbm.at[:, pl.ds(D + lo, n)],
                                  wk_v.at[:, pl.ds(lo, n)], sem.at[4 + j])
            for j, (lo, n) in enumerate(WKC)]
    c_wq = pltpu.make_async_copy(wqkv_hbm.at[:, pl.ds(0, D)], wq_v, sem.at[9])
    c_wv = pltpu.make_async_copy(wqkv_hbm.at[:, pl.ds(2 * D, D)], wv_v, sem.at[10])
    c_wo = pltpu.make_async_copy(wo_hbm, wo_v, sem.at[11])
    c_wg = pltpu.make_async_copy(wg_hbm, wg_v, sem.at[12])
    c_wu = pltpu.make_async_copy(wu_hbm, wu_v, sem.at[13])
    c_wd = pltpu.make_async_copy(wd_hbm, wd_v, sem.at[14])

    def rows(i):
        return pl.ds(i * TM, TM)

    def ln_x(lo, n):
        for c in range(n // CH):
            r = pl.ds(lo + c * CH, CH)
            xn_v[r, :] = _ln(x_v[r, :].astype(f32)).astype(bf16)

    def zsum(pkt, n, first):
        za = pkt[:, 0:128]
        for j in range(1, n // 128):
            za = za + pkt[:, j * 128:(j + 1) * 128]
        if first:
            zacc_v[...] = za
        else:
            zacc_v[...] += za

    def kt(lo, n):
        k_t = lax.dot_general(wkt_v[...], xn_v[pl.ds(lo, n), :], NT, preferred_element_type=f32)
        pkt = _phi(k_t)
        zsum(pkt, n, False)
        return pkt.astype(bf16)

    def g_part(lo, n, pkt, clo, chi):
        blk = _dot(pkt, xn_v[pl.ds(lo, n), clo:chi])
        if lo == 0:
            g_v[:, clo:chi] = blk
        else:
            g_v[:, clo:chi] += blk

    def q(i, lo=0, hi=D):
        qf = lax.dot_general(xn_v[rows(i), :], wqp_v[lo:hi, :], NT, preferred_element_type=f32)
        pqn_v[rows(i), lo:hi] = _phi(qf).astype(bf16)

    def q_norm(i, zrow, c0=0, c1=TM // CH):
        for c in range(c0, c1):
            rr = pl.ds(i * TM + c * CH, CH)
            pq = pqn_v[rr, :].astype(f32)
            t = pq[:, 0:128] * zrow[:, 0:128]
            for j in range(1, NL):
                t = t + pq[:, j * 128:(j + 1) * 128] * zrow[:, j * 128:(j + 1) * 128]
            t = t + pltpu.roll(t, 64, 1)
            t = t + pltpu.roll(t, 32, 1)
            r = 1.0 / (t + 1e-6)
            pqn_v[rr, :] = jnp.concatenate(
                [pq[:, j * 128:(j + 1) * 128] * r for j in range(NL)], axis=1).astype(bf16)

    def attn_mm(i):
        at_v[rows(i), :] = _dot(pqn_v[rows(i), :], m_v[...])

    def attn_post(i, c0=0, c1=TM // CH):
        for c in range(c0, c1):
            r = pl.ds(i * TM + c * CH, CH)
            h = x_v[r, :].astype(f32) + at_v[r, :]
            hn_v[r, :] = _ln(h).astype(bf16)

    c_x[0].start()
    for c in c_wk:
        c.start()
    for c in c_x[1:]:
        c.start()
    for c in (c_wq, c_wv, c_wo, c_wg, c_wu, c_wd):
        c.start()

    n0 = 256
    c_x[0].wait()
    ln_x(0, n0)
    pk_chunks = []
    for j, (lo, n) in enumerate(WKC):
        c_wk[j].wait()
        kj = _dot(xn_v[0:n0, :], wk_v[:, lo:lo + n])
        pk_chunks.append(_phi(kj).T)
    pkt = jnp.concatenate(pk_chunks, axis=0)
    zsum(pkt, n0, True)
    pk = pkt.astype(bf16)

    g_part(0, 256, pk, 0, GSPLIT)
    c_x[1].wait()
    wkt_v[...] = wk_v[...].astype(f32).T.astype(bf16)
    ln_x(256, 256)
    g_part(0, 256, pk, GSPLIT, D)
    pk = kt(256, 256)
    g_part(256, 256, pk, 0, GSPLIT)
    c_x[2].wait()
    ln_x(512, 512)
    g_part(256, 256, pk, GSPLIT, D)
    pk = kt(512, 512)
    g_part(512, 512, pk, 0, GSPLIT)
    c_x[3].wait()
    c_wq.wait()
    ln_x(1024, 512)
    wqt = wq_v[...].astype(f32).T
    for j in range(NL):
        t_v[j] = wqt[:, 128 * j:128 * (j + 1)]
    for d in range(DH):
        wqp_v[d * H:(d + 1) * H, :] = jnp.concatenate(
            [t_v[j, pl.ds(d, H, stride=DH), :] for j in range(NL)],
            axis=1).astype(bf16)
    g_part(512, 512, pk, GSPLIT, D)
    pk = kt(1024, 512)
    q(0)
    ln_x(1536, 512)
    g_part(1024, 512, pk, 0, D)
    pk = kt(1536, 512)
    q(1)
    g_part(1536, 512, pk, 0, GSPLIT)
    c_wv.wait()
    c_wo.wait()
    for d in range(DH):
        zp_v[d * H:(d + 1) * H, :] = zacc_v[pl.ds(d, H, stride=DH), :]
    zrow = jnp.sum(zp_v[...].T, axis=0, keepdims=True)
    g_part(1536, 512, pk, GSPLIT, D)

    kvs = []
    for j, (lo, hi) in enumerate(BANDS):
        n = hi - lo
        rr = lax.broadcasted_iota(jnp.int32, (n, 128), 0) + lo
        cc = lax.broadcasted_iota(jnp.int32, (n, 128), 1) + 128 * j
        kvj = _dot(g_v[lo:hi, :].astype(bf16), wv_v[:, 128 * j:128 * (j + 1)])
        kvs.append(jnp.where(_head_of(rr) == _head_of(cc), kvj, 0.0).astype(bf16))
    q(2, 0, 256)
    macc_v[...] = jnp.zeros_like(macc_v)
    for j, (lo, hi) in enumerate(BANDS):
        mj = _dot(kvs[j], wo_v[128 * j:128 * (j + 1), :])
        for jj in range(NL):
            macc_v[jj, lo:hi, :] += mj[:, 128 * jj:128 * (jj + 1)]
    c_wg.wait()
    c_wu.wait()
    c_wd.wait()
    for d in range(DH):
        m_v[d * H:(d + 1) * H, :] = jnp.concatenate(
            [macc_v[jj, pl.ds(d, H, stride=DH), :] for jj in range(NL)],
            axis=1).astype(bf16)
    q_norm(0, zrow)
    q(2, 256, D)
    attn_mm(0)
    q_norm(1, zrow)
    attn_post(0)
    attn_mm(1)

    def o_copy(lo, n, clo, cn, k):
        return pltpu.make_async_copy(
            obuf.at[pl.ds(lo, n), pl.ds(clo, cn)],
            out_hbm.at[pl.ds(lo, n), pl.ds(clo, cn)], osem.at[k])

    ocopies = []
    FC = 256
    NFC = F // FC
    NCH = TM // CH
    for i in range(NB):
        hn = hn_v[rows(i), :]
        a_parts = []
        if i == 0:
            q(3)
        for j in range(NFC):
            g = _dot(hn, wg_v[:, j * FC:(j + 1) * FC])
            if j == 0 and i >= 1:
                c = o_copy((i - 1) * TM, TM, 0, D, i - 1)
                c.start()
                ocopies.append(c)
            u = _dot(hn, wu_v[:, j * FC:(j + 1) * FC])
            a_parts.append((jnp.maximum(g, 0.0) * u).astype(bf16))
            if 1 <= j <= 4:
                lo, hi = (j - 1) * NCH // 4, j * NCH // 4
                if i + 1 < NB:
                    attn_post(i + 1, lo, hi)
                if i + 2 < NB:
                    q_norm(i + 2, zrow, lo, hi)
        a = jnp.concatenate(a_parts, axis=1)
        if i + 2 < NB:
            attn_mm(i + 2)
        if i + 1 < NB:
            y = _dot(a, wd_v[...])
            obuf[rows(i), :] = (x_v[rows(i), :].astype(f32) + at_v[rows(i), :] + y).astype(bf16)
        else:
            for k, (clo, cn) in enumerate(OC):
                y = _dot(a, wd_v[:, clo:clo + cn])
                obuf[rows(i), clo:clo + cn] = (
                    x_v[rows(i), clo:clo + cn].astype(f32) + at_v[rows(i), clo:clo + cn] + y
                ).astype(bf16)
                c = o_copy(i * TM, TM, clo, cn, NB - 1 + k)
                c.start()
                ocopies.append(c)
    for c in ocopies:
        c.wait()


@jax.jit
def pallas_sequential_preLN__linear_attn_block__glu_gated_reglu__prompt_kernel(
    A_x, A_wqkv, A_wo, B_x, B_W_gate, B_W_up, B_W_down,
):
    x = A_x.reshape(S, D)
    any_spec = pl.BlockSpec(memory_space=pl.ANY)
    out = pl.pallas_call(
        _kernel,
        out_shape=jax.ShapeDtypeStruct((S, D), bf16),
        in_specs=[any_spec] * 6,
        out_specs=any_spec,
        scratch_shapes=[
            pltpu.VMEM((S, D), bf16),
            pltpu.VMEM((D, D), bf16),
            pltpu.VMEM((D, D), bf16),
            pltpu.VMEM((D, D), bf16),
            pltpu.VMEM((D, D), bf16),
            pltpu.VMEM((D, F), bf16),
            pltpu.VMEM((D, F), bf16),
            pltpu.VMEM((F, D), bf16),
            pltpu.VMEM((D, D), bf16),
            pltpu.VMEM((NL, D, 128), f32),
            pltpu.VMEM((D, D), bf16),
            pltpu.VMEM((S, D), bf16),
            pltpu.VMEM((D, D), f32),
            pltpu.VMEM((D, 128), f32),
            pltpu.VMEM((D, 128), f32),
            pltpu.VMEM((NL, D, 128), f32),
            pltpu.VMEM((D, D), bf16),
            pltpu.VMEM((S, D), bf16),
            pltpu.VMEM((S, D), f32),
            pltpu.VMEM((S, D), bf16),
            pltpu.VMEM((S, D), bf16),
            pltpu.SemaphoreType.DMA((15,)),
            pltpu.SemaphoreType.DMA((NB + 2,)),
        ],
        compiler_params=pltpu.CompilerParams(vmem_limit_bytes=110 * 1024 * 1024),
    )(x, A_wqkv, A_wo, B_W_gate, B_W_up, B_W_down)
    return out.reshape(1, S, D)
```

```python
import jax
import jax.numpy as jnp
from jax import lax
import jax.experimental.pallas as pl
import jax.experimental.pallas.tpu as pltpu

S, D, F, H = 2048, 640, 1536, 32
DH = D // H
NL = D // 128
EPS = 1e-5
bf16 = jnp.bfloat16
f32 = jnp.float32

TQ = 512
TB = 128
NBB = S // TB
FC = 256
CH = 32
GB = 128
KR = 64
N0 = 256
GSPLIT = 256
BANDS = [(0, 144), (112, 272), (240, 400), (368, 528), (496, 640)]
WKC = [(0, 128), (128, 256), (384, 256)]
XP = [(0, 256), (256, 256), (512, 512), (1024, 1024)]
OC = [(0, 256), (256, 256), (512, 128)]
NT = (((1,), (1,)), ((), ()))


def _ln(x):
    mu = jnp.mean(x, axis=-1, keepdims=True)
    xc = x - mu
    var = jnp.mean(xc * xc, axis=-1, keepdims=True)
    return xc * lax.rsqrt(var + EPS)


def _phi(t):
    return jnp.where(t > 0, t + 1.0, jnp.exp(t)) + 1e-6


def _head_of(idx):
    return (idx * 3277) >> 16


def _dot(a, b):
    return jnp.dot(a, b, preferred_element_type=f32)


def _lane_tile_sum(v):
    acc = v[:, 0:128]
    for j in range(1, v.shape[1] // 128):
        acc = acc + v[:, j * 128:(j + 1) * 128]
    return acc


def _kernel(x_hbm, wqkv_hbm, wo_hbm, wg_hbm, wu_hbm, wd_hbm, out_hbm,
            x_v, wq_v, wk_v, wv_v, wo_v, wg_v, wu_v, wd_v,
            wkt_v, t_v, wqp_v, xn_v, g_v, zacc_v, zp_v, macc_v, m_v,
            pqn_v, at_v, hn_v, obuf,
            sem, osem):
    c_x = [pltpu.make_async_copy(x_hbm.at[pl.ds(lo, n), :], x_v.at[pl.ds(lo, n), :], sem.at[k])
           for k, (lo, n) in enumerate(XP)]
    c_wk = [pltpu.make_async_copy(wqkv_hbm.at[:, pl.ds(D + lo, n)],
                                  wk_v.at[:, pl.ds(lo, n)], sem.at[4 + j])
            for j, (lo, n) in enumerate(WKC)]
    c_wq = pltpu.make_async_copy(wqkv_hbm.at[:, pl.ds(0, D)], wq_v, sem.at[7])
    c_wv = pltpu.make_async_copy(wqkv_hbm.at[:, pl.ds(2 * D, D)], wv_v, sem.at[8])
    c_wo = pltpu.make_async_copy(wo_hbm, wo_v, sem.at[9])
    c_wg = pltpu.make_async_copy(wg_hbm, wg_v, sem.at[10])
    c_wu = pltpu.make_async_copy(wu_hbm, wu_v, sem.at[11])
    c_wd = pltpu.make_async_copy(wd_hbm, wd_v, sem.at[12])

    def o_copy(lo, n, clo, cn, k):
        return pltpu.make_async_copy(
            obuf.at[pl.ds(lo, n), pl.ds(clo, cn)],
            out_hbm.at[pl.ds(lo, n), pl.ds(clo, cn)], osem.at[k])

    def ln_x(lo, n):
        for c in range(n // CH):
            r = pl.ds(lo + c * CH, CH)
            xn_v[r, :] = _ln(x_v[r, :].astype(f32)).astype(bf16)

    def k_first(lo, n):
        kj = jnp.concatenate(
            [_dot(xn_v[c * KR:(c + 1) * KR, :], wk_v[:, lo:lo + n]) for c in range(N0 // KR)],
            axis=0)
        pkt = _phi(kj).T
        zacc_v[lo:lo + n, :] = _lane_tile_sum(pkt)
        return pkt.astype(bf16)

    def g_first(lo, n, pkt):
        for c in range(n // GB):
            g_v[lo + c * GB:lo + (c + 1) * GB, :] = _dot(
                pkt[c * GB:(c + 1) * GB, :], xn_v[0:N0, :])

    def kt(lo, n):
        pkt = _phi(lax.dot_general(wkt_v[...], xn_v[pl.ds(lo, n), :], NT,
                                   preferred_element_type=f32))
        zacc_v[...] += _lane_tile_sum(pkt)
        return pkt.astype(bf16)

    def g_part(lo, n, pkt, clo, chi):
        for c in range(D // GB):
            g_v[c * GB:(c + 1) * GB, clo:chi] += _dot(
                pkt[c * GB:(c + 1) * GB, :], xn_v[pl.ds(lo, n), clo:chi])

    def q(i, lo=0, hi=D):
        r = pl.ds(i * TQ, TQ)
        qf = lax.dot_general(xn_v[r, :], wqp_v[lo:hi, :], NT, preferred_element_type=f32)
        pqn_v[r, lo:hi] = _phi(qf).astype(bf16)

    def q_norm(lo, n, zrow):
        for c in range(n // CH):
            r = pl.ds(lo + c * CH, CH)
            pq = pqn_v[r, :].astype(f32)
            t = _lane_tile_sum(pq * zrow)
            t = t + pltpu.roll(t, 64, 1)
            t = t + pltpu.roll(t, 32, 1)
            inv = 1.0 / (t + 1e-6)
            pqn_v[r, :] = jnp.concatenate(
                [pq[:, j * 128:(j + 1) * 128] * inv for j in range(NL)], axis=1).astype(bf16)

    def attn_mm(lo, n):
        r = pl.ds(lo, n)
        at_v[r, :] = _dot(pqn_v[r, :], m_v[...])

    def attn_post(lo, n):
        for c in range(n // CH):
            r = pl.ds(lo + c * CH, CH)
            hn_v[r, :] = _ln(x_v[r, :].astype(f32) + at_v[r, :]).astype(bf16)

    def permute_rows(dst, src):
        for d in range(DH):
            dst[d * H:(d + 1) * H, :] = jnp.concatenate(
                [src[j, pl.ds(d, H, stride=DH), :] for j in range(NL)], axis=1).astype(bf16)

    c_x[0].start()
    for c in c_wk:
        c.start()
    for c in c_x[1:]:
        c.start()
    for c in (c_wq, c_wv, c_wo, c_wg, c_wu, c_wd):
        c.start()

    c_x[0].wait()
    ln_x(0, N0)
    prev = None
    for j, (lo, n) in enumerate(WKC):
        c_wk[j].wait()
        cur = (lo, n, k_first(lo, n))
        if prev is not None:
            g_first(*prev)
        prev = cur

    c_x[1].wait()
    wkt_v[...] = wk_v[...].astype(f32).T.astype(bf16)
    ln_x(256, 256)
    g_first(*prev)
    pk = kt(256, 256)
    g_part(256, 256, pk, 0, GSPLIT)
    c_x[2].wait()
    ln_x(512, 512)
    g_part(256, 256, pk, GSPLIT, D)
    pk = kt(512, 512)
    g_part(512, 512, pk, 0, GSPLIT)
    c_x[3].wait()
    c_wq.wait()
    ln_x(1024, 512)
    wqt = wq_v[...].astype(f32).T
    for j in range(NL):
        t_v[j] = wqt[:, 128 * j:128 * (j + 1)]
    permute_rows(wqp_v, t_v)
    g_part(512, 512, pk, GSPLIT, D)
    pk = kt(1024, 512)
    q(0)
    ln_x(1536, 512)
    g_part(1024, 512, pk, 0, D)
    pk = kt(1536, 512)
    q(1)
    g_part(1536, 512, pk, 0, GSPLIT)
    c_wv.wait()
    c_wo.wait()
    for d in range(DH):
        zp_v[d * H:(d + 1) * H, :] = zacc_v[pl.ds(d, H, stride=DH), :]
    zrow = jnp.sum(zp_v[...].T, axis=0, keepdims=True)
    g_part(1536, 512, pk, GSPLIT, D)

    kvs = []
    for j, (lo, hi) in enumerate(BANDS):
        n = hi - lo
        rr = lax.broadcasted_iota(jnp.int32, (n, 128), 0) + lo
        cc = lax.broadcasted_iota(jnp.int32, (n, 128), 1) + 128 * j
        kvj = _dot(g_v[lo:hi, :].astype(bf16), wv_v[:, 128 * j:128 * (j + 1)])
        kvs.append(jnp.where(_head_of(rr) == _head_of(cc), kvj, 0.0).astype(bf16))
    q(2, 0, 256)
    macc_v[...] = jnp.zeros_like(macc_v)
    for j, (lo, hi) in enumerate(BANDS):
        mj = _dot(kvs[j], wo_v[128 * j:128 * (j + 1), :])
        for jj in range(NL):
            macc_v[jj, lo:hi, :] += mj[:, 128 * jj:128 * (jj + 1)]
    c_wg.wait()
    c_wu.wait()
    c_wd.wait()
    permute_rows(m_v, macc_v)
    q_norm(0, TB, zrow)
    q(2, 256, D)
    attn_mm(0, TB)
    q_norm(TB, TB, zrow)
    attn_post(0, TB)
    attn_mm(TB, TB)

    ocopies = []
    for i in range(NBB):
        rr = pl.ds(i * TB, TB)
        hn = hn_v[rr, :]
        a_parts = []
        if i == 0:
            q(3)
        for j in range(F // FC):
            g = _dot(hn, wg_v[:, j * FC:(j + 1) * FC])
            if j == 0 and i >= 1:
                c = o_copy((i - 1) * TB, TB, 0, D, i - 1)
                c.start()
                ocopies.append(c)
            u = _dot(hn, wu_v[:, j * FC:(j + 1) * FC])
            a_parts.append((jnp.maximum(g, 0.0) * u).astype(bf16))
            if j == 1:
                if i + 1 < NBB:
                    attn_post((i + 1) * TB, TB)
                if i + 2 < NBB:
                    q_norm((i + 2) * TB, TB, zrow)
        a = jnp.concatenate(a_parts, axis=1)
        if i + 2 < NBB:
            attn_mm((i + 2) * TB, TB)
        if i + 1 < NBB:
            y = _dot(a, wd_v[...])
            obuf[rr, :] = (x_v[rr, :].astype(f32) + at_v[rr, :] + y).astype(bf16)
        else:
            for k, (clo, cn) in enumerate(OC):
                y = _dot(a, wd_v[:, clo:clo + cn])
                obuf[rr, clo:clo + cn] = (
                    x_v[rr, clo:clo + cn].astype(f32) + at_v[rr, clo:clo + cn] + y
                ).astype(bf16)
                c = o_copy(i * TB, TB, clo, cn, NBB - 1 + k)
                c.start()
                ocopies.append(c)
    for c in ocopies:
        c.wait()


@jax.jit
def pallas_sequential_preLN__linear_attn_block__glu_gated_reglu__prompt_kernel(
    A_x, A_wqkv, A_wo, B_x, B_W_gate, B_W_up, B_W_down,
):
    x = A_x.reshape(S, D)
    any_spec = pl.BlockSpec(memory_space=pl.ANY)
    out = pl.pallas_call(
        _kernel,
        out_shape=jax.ShapeDtypeStruct((S, D), bf16),
        in_specs=[any_spec] * 6,
        out_specs=any_spec,
        scratch_shapes=[
            pltpu.VMEM((S, D), bf16),
            pltpu.VMEM((D, D), bf16),
            pltpu.VMEM((D, D), bf16),
            pltpu.VMEM((D, D), bf16),
            pltpu.VMEM((D, D), bf16),
            pltpu.VMEM((D, F), bf16),
            pltpu.VMEM((D, F), bf16),
            pltpu.VMEM((F, D), bf16),
            pltpu.VMEM((D, D), bf16),
            pltpu.VMEM((NL, D, 128), f32),
            pltpu.VMEM((D, D), bf16),
            pltpu.VMEM((S, D), bf16),
            pltpu.VMEM((D, D), f32),
            pltpu.VMEM((D, 128), f32),
            pltpu.VMEM((D, 128), f32),
            pltpu.VMEM((NL, D, 128), f32),
            pltpu.VMEM((D, D), bf16),
            pltpu.VMEM((S, D), bf16),
            pltpu.VMEM((S, D), f32),
            pltpu.VMEM((S, D), bf16),
            pltpu.VMEM((S, D), bf16),
            pltpu.SemaphoreType.DMA((13,)),
            pltpu.SemaphoreType.DMA((NBB + 2,)),
        ],
        compiler_params=pltpu.CompilerParams(vmem_limit_bytes=110 * 1024 * 1024),
    )(x, A_wqkv, A_wo, B_W_gate, B_W_up, B_W_down)
    return out.reshape(1, S, D)
```

```python
import jax
import jax.numpy as jnp
from jax import lax
import jax.experimental.pallas as pl
import jax.experimental.pallas.tpu as pltpu

S, D, F, H = 2048, 640, 1536, 32
DH = D // H
NL = D // 128
EPS = 1e-5
bf16 = jnp.bfloat16
f32 = jnp.float32

TQ = 512
TB = 128
NBB = S // TB
FC = 256
CH = 32
GB = 128
KR = 128
N0 = 256
GSPLIT = 384
BANDS = [(0, 144), (112, 272), (240, 400), (368, 528), (496, 640)]
WKC = [(0, 128), (128, 256), (384, 256)]
XP = [(0, 256), (256, 384), (640, 384), (1024, 1024)]
OC = [(0, 256), (256, 256), (512, 128)]
NT = (((1,), (1,)), ((), ()))


def _ln(x):
    mu = jnp.mean(x, axis=-1, keepdims=True)
    xc = x - mu
    var = jnp.mean(xc * xc, axis=-1, keepdims=True)
    return xc * lax.rsqrt(var + EPS)


def _phi(t):
    return jnp.where(t > 0, t + 1.0, jnp.exp(t)) + 1e-6


def _head_of(idx):
    return (idx * 3277) >> 16


def _dot(a, b):
    return jnp.dot(a, b, preferred_element_type=f32)


def _lane_tile_sum(v):
    acc = v[:, 0:128]
    for j in range(1, v.shape[1] // 128):
        acc = acc + v[:, j * 128:(j + 1) * 128]
    return acc


def _kernel(x_hbm, wqkv_hbm, wo_hbm, wg_hbm, wu_hbm, wd_hbm, out_hbm,
            x_v, wq_v, wk_v, wv_v, wo_v, wg_v, wu_v, wd_v,
            wkt_v, t_v, wqp_v, xn_v, g_v, zacc_v, zp_v, macc_v, m_v,
            pqn_v, at_v, hn_v, obuf,
            sem, osem):
    c_x = [pltpu.make_async_copy(x_hbm.at[pl.ds(lo, n), :], x_v.at[pl.ds(lo, n), :], sem.at[k])
           for k, (lo, n) in enumerate(XP)]
    c_wk = [pltpu.make_async_copy(wqkv_hbm.at[:, pl.ds(D + lo, n)],
                                  wk_v.at[:, pl.ds(lo, n)], sem.at[4 + j])
            for j, (lo, n) in enumerate(WKC)]
    c_wq = pltpu.make_async_copy(wqkv_hbm.at[:, pl.ds(0, D)], wq_v, sem.at[7])
    c_wv = pltpu.make_async_copy(wqkv_hbm.at[:, pl.ds(2 * D, D)], wv_v, sem.at[8])
    c_wo = pltpu.make_async_copy(wo_hbm, wo_v, sem.at[9])
    c_wg = pltpu.make_async_copy(wg_hbm, wg_v, sem.at[10])
    c_wu = pltpu.make_async_copy(wu_hbm, wu_v, sem.at[11])
    c_wd = pltpu.make_async_copy(wd_hbm, wd_v, sem.at[12])

    def o_copy(lo, n, clo, cn, k):
        return pltpu.make_async_copy(
            obuf.at[pl.ds(lo, n), pl.ds(clo, cn)],
            out_hbm.at[pl.ds(lo, n), pl.ds(clo, cn)], osem.at[k])

    def ln_x(lo, n):
        for c in range(n // CH):
            r = pl.ds(lo + c * CH, CH)
            xn_v[r, :] = _ln(x_v[r, :].astype(f32)).astype(bf16)

    def k_first(lo, n):
        kj = jnp.concatenate(
            [_dot(xn_v[c * KR:(c + 1) * KR, :], wk_v[:, lo:lo + n]) for c in range(N0 // KR)],
            axis=0)
        pkt = _phi(kj).T
        zacc_v[lo:lo + n, :] = _lane_tile_sum(pkt)
        return pkt.astype(bf16)

    def g_first(lo, n, pkt):
        for c in range(n // GB):
            g_v[lo + c * GB:lo + (c + 1) * GB, :] = _dot(
                pkt[c * GB:(c + 1) * GB, :], xn_v[0:N0, :])

    def kt(lo, n):
        pkt = _phi(lax.dot_general(wkt_v[...], xn_v[pl.ds(lo, n), :], NT,
                                   preferred_element_type=f32))
        zacc_v[...] += _lane_tile_sum(pkt)
        return pkt.astype(bf16)

    def g_part(lo, n, pkt, clo, chi):
        for c in range(D // GB):
            g_v[c * GB:(c + 1) * GB, clo:chi] += _dot(
                pkt[c * GB:(c + 1) * GB, :], xn_v[pl.ds(lo, n), clo:chi])

    def q(i, lo=0, hi=D):
        r = pl.ds(i * TQ, TQ)
        qf = lax.dot_general(xn_v[r, :], wqp_v[lo:hi, :], NT, preferred_element_type=f32)
        pqn_v[r, lo:hi] = _phi(qf).astype(bf16)

    def q_norm(lo, n, zrow):
        for c in range(n // CH):
            r = pl.ds(lo + c * CH, CH)
            pq = pqn_v[r, :].astype(f32)
            t = _lane_tile_sum(pq * zrow)
            t = t + pltpu.roll(t, 64, 1)
            t = t + pltpu.roll(t, 32, 1)
            inv = 1.0 / (t + 1e-6)
            pqn_v[r, :] = jnp.concatenate(
                [pq[:, j * 128:(j + 1) * 128] * inv for j in range(NL)], axis=1).astype(bf16)

    def attn_mm(lo, n):
        r = pl.ds(lo, n)
        at_v[r, :] = _dot(pqn_v[r, :], m_v[...])

    def attn_post(lo, n):
        for c in range(n // CH):
            r = pl.ds(lo + c * CH, CH)
            hn_v[r, :] = _ln(x_v[r, :].astype(f32) + at_v[r, :]).astype(bf16)

    def permute_rows(dst, src):
        for d in range(DH):
            dst[d * H:(d + 1) * H, :] = jnp.concatenate(
                [src[j, pl.ds(d, H, stride=DH), :] for j in range(NL)], axis=1).astype(bf16)

    c_x[0].start()
    for c in c_wk:
        c.start()
    for c in c_x[1:]:
        c.start()
    for c in (c_wq, c_wv, c_wo, c_wg, c_wu, c_wd):
        c.start()

    c_x[0].wait()
    ln_x(0, N0)
    prev = None
    for j, (lo, n) in enumerate(WKC):
        c_wk[j].wait()
        cur = (lo, n, k_first(lo, n))
        if prev is not None:
            g_first(*prev)
        prev = cur

    c_x[1].wait()
    wkt_v[...] = wk_v[...].astype(f32).T.astype(bf16)
    ln_x(256, 384)
    g_first(*prev)
    pk = kt(256, 384)
    g_part(256, 384, pk, 0, GSPLIT)
    c_x[2].wait()
    c_x[3].wait()
    ln_x(640, 384)
    g_part(256, 384, pk, GSPLIT, D)
    pk = kt(640, 384)
    ln_x(1024, 512)
    g_part(640, 384, pk, 0, D)
    pk = kt(1024, 512)
    ln_x(1536, 512)
    g_part(1024, 512, pk, 0, D)
    pk = kt(1536, 512)
    g_part(1536, 512, pk, 0, GSPLIT)
    for c in (c_wq, c_wv, c_wo, c_wg, c_wu, c_wd):
        c.wait()
    wqt = wq_v[...].astype(f32).T
    for j in range(NL):
        t_v[j] = wqt[:, 128 * j:128 * (j + 1)]
    permute_rows(wqp_v, t_v)
    for d in range(DH):
        zp_v[d * H:(d + 1) * H, :] = zacc_v[pl.ds(d, H, stride=DH), :]
    zrow = jnp.sum(zp_v[...].T, axis=0, keepdims=True)
    g_part(1536, 512, pk, GSPLIT, D)

    kvs = []
    for j, (lo, hi) in enumerate(BANDS):
        n = hi - lo
        rr = lax.broadcasted_iota(jnp.int32, (n, 128), 0) + lo
        cc = lax.broadcasted_iota(jnp.int32, (n, 128), 1) + 128 * j
        kvj = _dot(g_v[lo:hi, :].astype(bf16), wv_v[:, 128 * j:128 * (j + 1)])
        kvs.append(jnp.where(_head_of(rr) == _head_of(cc), kvj, 0.0).astype(bf16))
    q(0)
    macc_v[...] = jnp.zeros_like(macc_v)
    for j, (lo, hi) in enumerate(BANDS):
        mj = _dot(kvs[j], wo_v[128 * j:128 * (j + 1), :])
        for jj in range(NL):
            macc_v[jj, lo:hi, :] += mj[:, 128 * jj:128 * (jj + 1)]
    permute_rows(m_v, macc_v)
    q_norm(0, TB, zrow)
    q(1)
    attn_mm(0, TB)
    q_norm(TB, TB, zrow)
    attn_post(0, TB)
    attn_mm(TB, TB)

    ocopies = []
    for i in range(NBB):
        rr = pl.ds(i * TB, TB)
        hn = hn_v[rr, :]
        a_parts = []
        if i == 0:
            q(2)
        if i == 3:
            q(3)
        for j in range(F // FC):
            g = _dot(hn, wg_v[:, j * FC:(j + 1) * FC])
            if j == 0 and i >= 1:
                c = o_copy((i - 1) * TB, TB, 0, D, i - 1)
                c.start()
                ocopies.append(c)
            u = _dot(hn, wu_v[:, j * FC:(j + 1) * FC])
            a_parts.append((jnp.maximum(g, 0.0) * u).astype(bf16))
            if j == 1:
                if i + 1 < NBB:
                    attn_post((i + 1) * TB, TB)
                if i + 2 < NBB:
                    q_norm((i + 2) * TB, TB, zrow)
        a = jnp.concatenate(a_parts, axis=1)
        if i + 2 < NBB:
            attn_mm((i + 2) * TB, TB)
        if i + 1 < NBB:
            y = _dot(a, wd_v[...])
            obuf[rr, :] = (x_v[rr, :].astype(f32) + at_v[rr, :] + y).astype(bf16)
        else:
            for k, (clo, cn) in enumerate(OC):
                y = _dot(a, wd_v[:, clo:clo + cn])
                obuf[rr, clo:clo + cn] = (
                    x_v[rr, clo:clo + cn].astype(f32) + at_v[rr, clo:clo + cn] + y
                ).astype(bf16)
                c = o_copy(i * TB, TB, clo, cn, NBB - 1 + k)
                c.start()
                ocopies.append(c)
    for c in ocopies:
        c.wait()


@jax.jit
def pallas_sequential_preLN__linear_attn_block__glu_gated_reglu__prompt_kernel(
    A_x, A_wqkv, A_wo, B_x, B_W_gate, B_W_up, B_W_down,
):
    x = A_x.reshape(S, D)
    any_spec = pl.BlockSpec(memory_space=pl.ANY)
    out = pl.pallas_call(
        _kernel,
        out_shape=jax.ShapeDtypeStruct((S, D), bf16),
        in_specs=[any_spec] * 6,
        out_specs=any_spec,
        scratch_shapes=[
            pltpu.VMEM((S, D), bf16),
            pltpu.VMEM((D, D), bf16),
            pltpu.VMEM((D, D), bf16),
            pltpu.VMEM((D, D), bf16),
            pltpu.VMEM((D, D), bf16),
            pltpu.VMEM((D, F), bf16),
            pltpu.VMEM((D, F), bf16),
            pltpu.VMEM((F, D), bf16),
            pltpu.VMEM((D, D), bf16),
            pltpu.VMEM((NL, D, 128), f32),
            pltpu.VMEM((D, D), bf16),
            pltpu.VMEM((S, D), bf16),
            pltpu.VMEM((D, D), f32),
            pltpu.VMEM((D, 128), f32),
            pltpu.VMEM((D, 128), f32),
            pltpu.VMEM((NL, D, 128), f32),
            pltpu.VMEM((D, D), bf16),
            pltpu.VMEM((S, D), bf16),
            pltpu.VMEM((S, D), f32),
            pltpu.VMEM((S, D), bf16),
            pltpu.VMEM((S, D), bf16),
            pltpu.SemaphoreType.DMA((13,)),
            pltpu.SemaphoreType.DMA((NBB + 2,)),
        ],
        compiler_params=pltpu.CompilerParams(vmem_limit_bytes=110 * 1024 * 1024),
    )(x, A_wqkv, A_wo, B_W_gate, B_W_up, B_W_down)
    return out.reshape(1, S, D)
```

```python
import jax
import jax.numpy as jnp
from jax import lax
import jax.experimental.pallas as pl
import jax.experimental.pallas.tpu as pltpu

S, D, F, H = 2048, 640, 1536, 32
DH = D // H
NL = D // 128
EPS = 1e-5
bf16 = jnp.bfloat16
f32 = jnp.float32

TQ = 512
TB = 128
NBB = S // TB
FC = 256
CH = 32
GB = 128
KR = 128
N0 = 256
GSPLIT = 384
BANDS = [(0, 144), (112, 272), (240, 400), (368, 528), (496, 640)]
WKC = [(0, 128), (128, 256), (384, 256)]
XP = [(0, 256), (256, 384), (640, 1408)]
OC = [(0, 256), (256, 256), (512, 128)]
NT = (((1,), (1,)), ((), ()))


def _ln(x):
    mu = jnp.mean(x, axis=-1, keepdims=True)
    xc = x - mu
    var = jnp.mean(xc * xc, axis=-1, keepdims=True)
    return xc * lax.rsqrt(var + EPS)


def _phi(t):
    return jnp.where(t > 0, t + 1.0, jnp.exp(t)) + 1e-6


def _head_of(idx):
    return (idx * 3277) >> 16


def _dot(a, b):
    return jnp.dot(a, b, preferred_element_type=f32)


def _lane_tile_sum(v):
    acc = v[:, 0:128]
    for j in range(1, v.shape[1] // 128):
        acc = acc + v[:, j * 128:(j + 1) * 128]
    return acc


def _kernel(x_hbm, wqkv_hbm, wo_hbm, wg_hbm, wu_hbm, wd_hbm, out_hbm,
            x_v, wq_v, wk_v, wv_v, wo_v, wg_v, wu_v, wd_v,
            wkt_v, t_v, wqp_v, xn_v, g_v, zacc_v, zp_v, macc_v, m_v,
            pqn_v, at_v, hn_v, obuf,
            sem, osem):
    c_x = [pltpu.make_async_copy(x_hbm.at[pl.ds(lo, n), :], x_v.at[pl.ds(lo, n), :], sem.at[k])
           for k, (lo, n) in enumerate(XP)]
    c_wk = [pltpu.make_async_copy(wqkv_hbm.at[:, pl.ds(D + lo, n)],
                                  wk_v.at[:, pl.ds(lo, n)], sem.at[3 + j])
            for j, (lo, n) in enumerate(WKC)]
    c_wq = pltpu.make_async_copy(wqkv_hbm.at[:, pl.ds(0, D)], wq_v, sem.at[6])
    c_wv = pltpu.make_async_copy(wqkv_hbm.at[:, pl.ds(2 * D, D)], wv_v, sem.at[6])
    c_wo = pltpu.make_async_copy(wo_hbm, wo_v, sem.at[6])
    c_wg = pltpu.make_async_copy(wg_hbm, wg_v, sem.at[6])
    c_wu = pltpu.make_async_copy(wu_hbm, wu_v, sem.at[6])
    c_wd = pltpu.make_async_copy(wd_hbm, wd_v, sem.at[6])

    def o_copy(lo, n, clo, cn):
        return pltpu.make_async_copy(
            obuf.at[pl.ds(lo, n), pl.ds(clo, cn)],
            out_hbm.at[pl.ds(lo, n), pl.ds(clo, cn)], osem.at[0])

    def ln_x(lo, n):
        for c in range(n // CH):
            r = pl.ds(lo + c * CH, CH)
            xn_v[r, :] = _ln(x_v[r, :].astype(f32)).astype(bf16)

    def k_first(lo, n):
        kj = jnp.concatenate(
            [_dot(xn_v[c * KR:(c + 1) * KR, :], wk_v[:, lo:lo + n]) for c in range(N0 // KR)],
            axis=0)
        pkt = _phi(kj).T
        zacc_v[lo:lo + n, :] = _lane_tile_sum(pkt)
        return pkt.astype(bf16)

    def g_first(lo, n, pkt):
        for c in range(n // GB):
            g_v[lo + c * GB:lo + (c + 1) * GB, :] = _dot(
                pkt[c * GB:(c + 1) * GB, :], xn_v[0:N0, :])

    def kt(lo, n):
        pkt = _phi(lax.dot_general(wkt_v[...], xn_v[pl.ds(lo, n), :], NT,
                                   preferred_element_type=f32))
        zacc_v[...] += _lane_tile_sum(pkt)
        return pkt.astype(bf16)

    def g_part(lo, n, pkt, clo, chi):
        for c in range(D // GB):
            g_v[c * GB:(c + 1) * GB, clo:chi] += _dot(
                pkt[c * GB:(c + 1) * GB, :], xn_v[pl.ds(lo, n), clo:chi])

    def q(i, lo=0, hi=D):
        r = pl.ds(i * TQ, TQ)
        qf = lax.dot_general(xn_v[r, :], wqp_v[lo:hi, :], NT, preferred_element_type=f32)
        pqn_v[r, lo:hi] = _phi(qf).astype(bf16)

    def q_norm(lo, n, zrow):
        for c in range(n // CH):
            r = pl.ds(lo + c * CH, CH)
            pq = pqn_v[r, :].astype(f32)
            t = _lane_tile_sum(pq * zrow)
            t = t + pltpu.roll(t, 64, 1)
            t = t + pltpu.roll(t, 32, 1)
            inv = 1.0 / (t + 1e-6)
            pqn_v[r, :] = jnp.concatenate(
                [pq[:, j * 128:(j + 1) * 128] * inv for j in range(NL)], axis=1).astype(bf16)

    def attn_mm(lo, n):
        r = pl.ds(lo, n)
        at_v[r, :] = _dot(pqn_v[r, :], m_v[...])

    def attn_post(lo, n):
        for c in range(n // CH):
            r = pl.ds(lo + c * CH, CH)
            hn_v[r, :] = _ln(x_v[r, :].astype(f32) + at_v[r, :]).astype(bf16)

    def permute_rows(dst, src):
        for d in range(DH):
            dst[d * H:(d + 1) * H, :] = jnp.concatenate(
                [src[j, pl.ds(d, H, stride=DH), :] for j in range(NL)], axis=1).astype(bf16)

    c_x[0].start()
    for c in c_wk:
        c.start()
    for c in c_x[1:]:
        c.start()
    for c in (c_wq, c_wv, c_wo, c_wg, c_wu, c_wd):
        c.start()

    c_x[0].wait()
    ln_x(0, N0)
    prev = None
    for j, (lo, n) in enumerate(WKC):
        c_wk[j].wait()
        cur = (lo, n, k_first(lo, n))
        if prev is not None:
            g_first(*prev)
        prev = cur

    c_x[1].wait()
    wkt_v[...] = wk_v[...].astype(f32).T.astype(bf16)
    ln_x(256, 384)
    g_first(*prev)
    pk = kt(256, 384)
    g_part(256, 384, pk, 0, GSPLIT)
    c_x[2].wait()
    ln_x(640, 384)
    g_part(256, 384, pk, GSPLIT, D)
    pk = kt(640, 384)
    ln_x(1024, 512)
    g_part(640, 384, pk, 0, D)
    pk = kt(1024, 512)
    ln_x(1536, 512)
    g_part(1024, 512, pk, 0, D)
    pk = kt(1536, 512)
    g_part(1536, 512, pk, 0, GSPLIT)
    for c in (c_wq, c_wv, c_wo, c_wg, c_wu, c_wd):
        c.wait()
    wqt = wq_v[...].astype(f32).T
    for j in range(NL):
        t_v[j] = wqt[:, 128 * j:128 * (j + 1)]
    permute_rows(wqp_v, t_v)
    for d in range(DH):
        zp_v[d * H:(d + 1) * H, :] = zacc_v[pl.ds(d, H, stride=DH), :]
    zrow = jnp.sum(zp_v[...].T, axis=0, keepdims=True)
    g_part(1536, 512, pk, GSPLIT, D)

    kvs = []
    for j, (lo, hi) in enumerate(BANDS):
        n = hi - lo
        rr = lax.broadcasted_iota(jnp.int32, (n, 128), 0) + lo
        cc = lax.broadcasted_iota(jnp.int32, (n, 128), 1) + 128 * j
        kvj = _dot(g_v[lo:hi, :].astype(bf16), wv_v[:, 128 * j:128 * (j + 1)])
        kvs.append(jnp.where(_head_of(rr) == _head_of(cc), kvj, 0.0).astype(bf16))
    q(0)
    macc_v[...] = jnp.zeros_like(macc_v)
    for j, (lo, hi) in enumerate(BANDS):
        mj = _dot(kvs[j], wo_v[128 * j:128 * (j + 1), :])
        for jj in range(NL):
            macc_v[jj, lo:hi, :] += mj[:, 128 * jj:128 * (jj + 1)]
    permute_rows(m_v, macc_v)
    q_norm(0, TB, zrow)
    q(1)
    attn_mm(0, TB)
    q_norm(TB, TB, zrow)
    attn_post(0, TB)
    attn_mm(TB, TB)

    for i in range(NBB):
        rr = pl.ds(i * TB, TB)
        hn = hn_v[rr, :]
        a_parts = []
        if i == 0:
            q(2)
        if i == 3:
            q(3)
        for j in range(F // FC):
            g = _dot(hn, wg_v[:, j * FC:(j + 1) * FC])
            if j == 0 and i >= 1:
                o_copy((i - 1) * TB, TB, 0, D).start()
            u = _dot(hn, wu_v[:, j * FC:(j + 1) * FC])
            a_parts.append((jnp.maximum(g, 0.0) * u).astype(bf16))
            if j == 1:
                if i + 1 < NBB:
                    attn_post((i + 1) * TB, TB)
                if i + 2 < NBB:
                    q_norm((i + 2) * TB, TB, zrow)
        a = jnp.concatenate(a_parts, axis=1)
        if i + 2 < NBB:
            attn_mm((i + 2) * TB, TB)
        if i + 1 < NBB:
            y = _dot(a, wd_v[...])
            obuf[rr, :] = (x_v[rr, :].astype(f32) + at_v[rr, :] + y).astype(bf16)
        else:
            for clo, cn in OC:
                y = _dot(a, wd_v[:, clo:clo + cn])
                obuf[rr, clo:clo + cn] = (
                    x_v[rr, clo:clo + cn].astype(f32) + at_v[rr, clo:clo + cn] + y
                ).astype(bf16)
                o_copy(i * TB, TB, clo, cn).start()
    o_copy(0, S, 0, D).wait()


@jax.jit
def pallas_sequential_preLN__linear_attn_block__glu_gated_reglu__prompt_kernel(
    A_x, A_wqkv, A_wo, B_x, B_W_gate, B_W_up, B_W_down,
):
    x = A_x.reshape(S, D)
    any_spec = pl.BlockSpec(memory_space=pl.ANY)
    out = pl.pallas_call(
        _kernel,
        out_shape=jax.ShapeDtypeStruct((S, D), bf16),
        in_specs=[any_spec] * 6,
        out_specs=any_spec,
        scratch_shapes=[
            pltpu.VMEM((S, D), bf16),
            pltpu.VMEM((D, D), bf16),
            pltpu.VMEM((D, D), bf16),
            pltpu.VMEM((D, D), bf16),
            pltpu.VMEM((D, D), bf16),
            pltpu.VMEM((D, F), bf16),
            pltpu.VMEM((D, F), bf16),
            pltpu.VMEM((F, D), bf16),
            pltpu.VMEM((D, D), bf16),
            pltpu.VMEM((NL, D, 128), f32),
            pltpu.VMEM((D, D), bf16),
            pltpu.VMEM((S, D), bf16),
            pltpu.VMEM((D, D), f32),
            pltpu.VMEM((D, 128), f32),
            pltpu.VMEM((D, 128), f32),
            pltpu.VMEM((NL, D, 128), f32),
            pltpu.VMEM((D, D), bf16),
            pltpu.VMEM((S, D), bf16),
            pltpu.VMEM((S, D), f32),
            pltpu.VMEM((S, D), bf16),
            pltpu.VMEM((S, D), bf16),
            pltpu.SemaphoreType.DMA((7,)),
            pltpu.SemaphoreType.DMA((1,)),
        ],
        compiler_params=pltpu.CompilerParams(vmem_limit_bytes=110 * 1024 * 1024),
    )(x, A_wqkv, A_wo, B_W_gate, B_W_up, B_W_down)
    return out.reshape(1, S, D)
```

```python
import jax
import jax.numpy as jnp
from jax import lax
import jax.experimental.pallas as pl
import jax.experimental.pallas.tpu as pltpu

S, D, F, H = 2048, 640, 1536, 32
DH = D // H
NL = D // 128
EPS = 1e-5
bf16 = jnp.bfloat16
f32 = jnp.float32

TQ = 512
TB = 128
NBB = S // TB
FC = 256
QB = 128
CH = 32
GB = 128
KR = 128
N0 = 256
GSPLIT = 384
BANDS = [(0, 144), (112, 272), (240, 400), (368, 528), (496, 640)]
WKC = [(0, 128), (128, 256), (384, 256)]
XP = [(0, 256), (256, 384), (640, 1408)]
OC = [(0, 256), (256, 256), (512, 128)]
NT = (((1,), (1,)), ((), ()))


def _ln(x):
    mu = jnp.mean(x, axis=-1, keepdims=True)
    xc = x - mu
    var = jnp.mean(xc * xc, axis=-1, keepdims=True)
    return xc * lax.rsqrt(var + EPS)


def _phi(t):
    return jnp.where(t > 0, t + 1.0, jnp.exp(t)) + 1e-6


def _head_of(idx):
    return (idx * 3277) >> 16


def _dot(a, b):
    return jnp.dot(a, b, preferred_element_type=f32)


def _pk(v):
    return pltpu.bitcast(v, jnp.uint32)


def _ld(ref, lo, n, clo=0, chi=D):
    return pltpu.bitcast(ref[pl.ds(lo // 2, n // 2), clo:chi], bf16)


def _st(ref, lo, v, clo=0, chi=D):
    ref[pl.ds(lo // 2, v.shape[0] // 2), clo:chi] = _pk(v)


def _lane_tile_sum(v):
    acc = v[:, 0:128]
    for j in range(1, v.shape[1] // 128):
        acc = acc + v[:, j * 128:(j + 1) * 128]
    return acc


def _kernel(x_hbm, wqkv_hbm, wo_hbm, wg_hbm, wu_hbm, wd_hbm, out_hbm,
            x_v, wq_v, wk_v, wv_v, wo_v, wg_v, wu_v, wd_v,
            wkt_v, t_v, wqp_v, xn_v, g_v, zacc_v, zp_v, macc_v, m_v,
            pqn_v, at_v, hn_v, obuf,
            sem, osem):
    c_x = [pltpu.make_async_copy(x_hbm.at[pl.ds(lo, n), :], x_v.at[pl.ds(lo, n), :], sem.at[k])
           for k, (lo, n) in enumerate(XP)]
    c_wk = [pltpu.make_async_copy(wqkv_hbm.at[:, pl.ds(D + lo, n)],
                                  wk_v.at[:, pl.ds(lo, n)], sem.at[3 + j])
            for j, (lo, n) in enumerate(WKC)]
    c_wq = pltpu.make_async_copy(wqkv_hbm.at[:, pl.ds(0, D)], wq_v, sem.at[6])
    c_wv = pltpu.make_async_copy(wqkv_hbm.at[:, pl.ds(2 * D, D)], wv_v, sem.at[6])
    c_wo = pltpu.make_async_copy(wo_hbm, wo_v, sem.at[6])
    c_wg = pltpu.make_async_copy(wg_hbm, wg_v, sem.at[6])
    c_wu = pltpu.make_async_copy(wu_hbm, wu_v, sem.at[6])
    c_wd = pltpu.make_async_copy(wd_hbm, wd_v, sem.at[6])

    def o_copy(lo, n, clo, cn):
        return pltpu.make_async_copy(
            obuf.at[pl.ds(lo, n), pl.ds(clo, cn)],
            out_hbm.at[pl.ds(lo, n), pl.ds(clo, cn)], osem.at[0])

    def ln_x(lo, n):
        for c in range(n // CH):
            r = pl.ds(lo + c * CH, CH)
            _st(xn_v, lo + c * CH, _ln(x_v[r, :].astype(f32)).astype(bf16))

    def k_first(lo, n):
        kj = jnp.concatenate(
            [_dot(_ld(xn_v, c * KR, KR), wk_v[:, lo:lo + n]) for c in range(N0 // KR)],
            axis=0)
        pkt = _phi(kj).T
        zacc_v[lo:lo + n, :] = _lane_tile_sum(pkt)
        return pkt.astype(bf16)

    def g_first(lo, n, pkt):
        for c in range(n // GB):
            g_v[lo + c * GB:lo + (c + 1) * GB, :] = _dot(
                pkt[c * GB:(c + 1) * GB, :], _ld(xn_v, 0, N0))

    def kt(lo, n):
        pkt = _phi(lax.dot_general(_ld(wkt_v, 0, D), _ld(xn_v, lo, n), NT,
                                   preferred_element_type=f32))
        zacc_v[...] += _lane_tile_sum(pkt)
        return pkt.astype(bf16)

    def g_part(lo, n, pkt, clo, chi):
        for c in range(D // GB):
            g_v[c * GB:(c + 1) * GB, clo:chi] += _dot(
                pkt[c * GB:(c + 1) * GB, :], _ld(xn_v, lo, n, clo, chi))

    def q(i, lo=0, hi=D):
        for c in range(TQ // QB):
            qf = lax.dot_general(_ld(xn_v, i * TQ + c * QB, QB), _ld(wqp_v, lo, hi - lo), NT,
                                 preferred_element_type=f32)
            _st(pqn_v, i * TQ + c * QB, _phi(qf).astype(bf16), lo, hi)

    def q_norm(lo, n, zrow):
        for c in range(n // CH):
            pq = _ld(pqn_v, lo + c * CH, CH).astype(f32)
            t = _lane_tile_sum(pq * zrow)
            t = t + pltpu.roll(t, 64, 1)
            t = t + pltpu.roll(t, 32, 1)
            inv = 1.0 / (t + 1e-6)
            _st(pqn_v, lo + c * CH, jnp.concatenate(
                [pq[:, j * 128:(j + 1) * 128] * inv for j in range(NL)], axis=1).astype(bf16))

    def attn_mm(lo, n):
        r = pl.ds(lo, n)
        at_v[r, :] = _dot(_ld(pqn_v, lo, n), _ld(m_v, 0, D))

    def attn_post(lo, n):
        for c in range(n // CH):
            r = pl.ds(lo + c * CH, CH)
            _st(hn_v, lo + c * CH, _ln(x_v[r, :].astype(f32) + at_v[r, :]).astype(bf16))

    def permute_rows(dst, src):
        for d in range(DH):
            _st(dst, d * H, jnp.concatenate(
                [src[j, pl.ds(d, H, stride=DH), :] for j in range(NL)], axis=1).astype(bf16))

    c_x[0].start()
    for c in c_wk:
        c.start()
    for c in c_x[1:]:
        c.start()
    for c in (c_wq, c_wv, c_wo, c_wg, c_wu, c_wd):
        c.start()

    c_x[0].wait()
    ln_x(0, N0)
    prev = None
    for j, (lo, n) in enumerate(WKC):
        c_wk[j].wait()
        cur = (lo, n, k_first(lo, n))
        if prev is not None:
            g_first(*prev)
        prev = cur

    c_x[1].wait()
    _st(wkt_v, 0, wk_v[...].astype(f32).T.astype(bf16))
    ln_x(256, 384)
    g_first(*prev)
    pk = kt(256, 384)
    g_part(256, 384, pk, 0, GSPLIT)
    c_x[2].wait()
    ln_x(640, 384)
    g_part(256, 384, pk, GSPLIT, D)
    pk = kt(640, 384)
    ln_x(1024, 512)
    g_part(640, 384, pk, 0, D)
    pk = kt(1024, 512)
    ln_x(1536, 512)
    g_part(1024, 512, pk, 0, D)
    pk = kt(1536, 512)
    g_part(1536, 512, pk, 0, GSPLIT)
    for c in (c_wq, c_wv, c_wo, c_wg, c_wu, c_wd):
        c.wait()
    wqt = wq_v[...].astype(f32).T
    for j in range(NL):
        t_v[j] = wqt[:, 128 * j:128 * (j + 1)]
    permute_rows(wqp_v, t_v)
    for d in range(DH):
        zp_v[d * H:(d + 1) * H, :] = zacc_v[pl.ds(d, H, stride=DH), :]
    zrow = jnp.sum(zp_v[...].T, axis=0, keepdims=True)
    g_part(1536, 512, pk, GSPLIT, D)

    kvs = []
    for j, (lo, hi) in enumerate(BANDS):
        n = hi - lo
        rr = lax.broadcasted_iota(jnp.int32, (n, 128), 0) + lo
        cc = lax.broadcasted_iota(jnp.int32, (n, 128), 1) + 128 * j
        kvj = _dot(g_v[lo:hi, :].astype(bf16), wv_v[:, 128 * j:128 * (j + 1)])
        kvs.append(jnp.where(_head_of(rr) == _head_of(cc), kvj, 0.0).astype(bf16))
    q(0)
    macc_v[...] = jnp.zeros_like(macc_v)
    for j, (lo, hi) in enumerate(BANDS):
        mj = _dot(kvs[j], wo_v[128 * j:128 * (j + 1), :])
        for jj in range(NL):
            macc_v[jj, lo:hi, :] += mj[:, 128 * jj:128 * (jj + 1)]
    permute_rows(m_v, macc_v)
    q_norm(0, TB, zrow)
    q(1)
    attn_mm(0, TB)
    q_norm(TB, TB, zrow)
    attn_post(0, TB)
    attn_mm(TB, TB)

    for i in range(NBB):
        rr = pl.ds(i * TB, TB)
        hn = _ld(hn_v, i * TB, TB)
        a_parts = []
        if i == 0:
            q(2)
        if i == 3:
            q(3)
        for j in range(F // FC):
            g = _dot(hn, wg_v[:, j * FC:(j + 1) * FC])
            if j == 0 and i >= 1:
                o_copy((i - 1) * TB, TB, 0, D).start()
            u = _dot(hn, wu_v[:, j * FC:(j + 1) * FC])
            a_parts.append((jnp.maximum(g, 0.0) * u).astype(bf16))
            if j == 1:
                if i + 1 < NBB:
                    attn_post((i + 1) * TB, TB)
                if i + 2 < NBB:
                    q_norm((i + 2) * TB, TB, zrow)
        a = jnp.concatenate(a_parts, axis=1)
        if i + 2 < NBB:
            attn_mm((i + 2) * TB, TB)
        if i + 1 < NBB:
            y = _dot(a, wd_v[...])
            obuf[rr, :] = (x_v[rr, :].astype(f32) + at_v[rr, :] + y).astype(bf16)
        else:
            for clo, cn in OC:
                y = _dot(a, wd_v[:, clo:clo + cn])
                obuf[rr, clo:clo + cn] = (
                    x_v[rr, clo:clo + cn].astype(f32) + at_v[rr, clo:clo + cn] + y
                ).astype(bf16)
                o_copy(i * TB, TB, clo, cn).start()
    o_copy(0, S, 0, D).wait()


@jax.jit
def pallas_sequential_preLN__linear_attn_block__glu_gated_reglu__prompt_kernel(
    A_x, A_wqkv, A_wo, B_x, B_W_gate, B_W_up, B_W_down,
):
    x = A_x.reshape(S, D)
    any_spec = pl.BlockSpec(memory_space=pl.ANY)
    out = pl.pallas_call(
        _kernel,
        out_shape=jax.ShapeDtypeStruct((S, D), bf16),
        in_specs=[any_spec] * 6,
        out_specs=any_spec,
        scratch_shapes=[
            pltpu.VMEM((S, D), bf16),
            pltpu.VMEM((D, D), bf16),
            pltpu.VMEM((D, D), bf16),
            pltpu.VMEM((D, D), bf16),
            pltpu.VMEM((D, D), bf16),
            pltpu.VMEM((D, F), bf16),
            pltpu.VMEM((D, F), bf16),
            pltpu.VMEM((F, D), bf16),
            pltpu.VMEM((D // 2, D), jnp.uint32),
            pltpu.VMEM((NL, D, 128), f32),
            pltpu.VMEM((D // 2, D), jnp.uint32),
            pltpu.VMEM((S // 2, D), jnp.uint32),
            pltpu.VMEM((D, D), f32),
            pltpu.VMEM((D, 128), f32),
            pltpu.VMEM((D, 128), f32),
            pltpu.VMEM((NL, D, 128), f32),
            pltpu.VMEM((D // 2, D), jnp.uint32),
            pltpu.VMEM((S // 2, D), jnp.uint32),
            pltpu.VMEM((S, D), f32),
            pltpu.VMEM((S // 2, D), jnp.uint32),
            pltpu.VMEM((S, D), bf16),
            pltpu.SemaphoreType.DMA((7,)),
            pltpu.SemaphoreType.DMA((1,)),
        ],
        compiler_params=pltpu.CompilerParams(vmem_limit_bytes=110 * 1024 * 1024),
    )(x, A_wqkv, A_wo, B_W_gate, B_W_up, B_W_down)
    return out.reshape(1, S, D)
```
